```python
import os as _os
_os.environ.setdefault("JAX_PLATFORMS", "cpu")
import jax
import jax.numpy as jnp

def _softmax(x, axis=-1):
    return jax.nn.softmax(x, axis=axis)
def _gelu(x):
    return jax.nn.gelu(x, approximate=True)
def _silu(x):
    return jax.nn.silu(x)
def _sigmoid(x):
    return jax.nn.sigmoid(x)
def _layernorm(x, axis=-1, eps=1e-5):
    m = jnp.mean(x, axis=axis, keepdims=True)
    v = jnp.var(x, axis=axis, keepdims=True)
    return (x - m) / jnp.sqrt(v + eps)
def _scatter_add(tgt, idx, src, axis=0):
    return tgt.at[idx].add(src)
def _segment_sum(src, seg, n):
    return jax.ops.segment_sum(src, seg, n)
class _Rng:
    def __init__(self, key):
        self._k = key
    def _next(self):
        self._k, sub = jax.random.split(self._k)
        return sub
    def normal(self, shape):
        return jax.random.normal(self._next(), shape, dtype=jnp.bfloat16)
    def randint(self, lo, hi, shape):
        return jax.random.randint(self._next(), shape, lo, hi, dtype=jnp.int32)
    def uniform(self, shape, lo=0.0, hi=1.0):
        return jax.random.uniform(self._next(), shape, jnp.bfloat16, lo, hi)
    def permutation(self, n):
        return jax.random.permutation(self._next(), n)


kernel_name = 'standalone__linear_kernel_hedgehog__prompt'

def setup_inputs():
    _rng = _Rng(jax.random.key(int.from_bytes(__import__("os").urandom(4), "little")))
    _w = (lambda a: (lambda t: t.astype(jnp.bfloat16) if jnp.issubdtype(t.dtype, jnp.floating) else t)(jnp.asarray(a)))
    B, S, D, H = 1, 2048, 1024, 32
    Dh = D // H
    return {
        "x": _w((lambda *s: _rng.normal(s) * 0.4)(B, S, D)),
        "wqkv": _w((lambda *s: _rng.normal(s) * 0.4)(D, 3 * D)),
        "w_phi": _w((lambda *s: _rng.normal(s) * 0.4)(H, Dh, Dh) * (Dh ** -0.5)),
        "wo": _w((lambda *s: _rng.normal(s) * 0.05)(D, D)),
    }

def reference(x, wqkv, w_phi, wo):
    B, S, D = x.shape
    H = 32; Dh = D // H
    qkv = (lambda x, *d: x.transpose(*d))((x @ wqkv).reshape(B, S, 3, H, Dh), 2, 0, 3, 1, 4)
    q, k, v = qkv[0], qkv[1], qkv[2]
    pq = jnp.einsum("bhsd,hdf->bhsf", q, w_phi)
    pk = jnp.einsum("bhsd,hdf->bhsf", k, w_phi)
    phi_q = jnp.concatenate([_softmax(pq, axis=-1), _softmax(-pq, axis=-1)], axis=-1)
    phi_k = jnp.concatenate([_softmax(pk, axis=-1), _softmax(-pk, axis=-1)], axis=-1)
    kv = jnp.einsum("bhsf,bhsd->bhfd", phi_k, v)
    z  = jnp.einsum("bhsf->bhf", phi_k)
    num = jnp.einsum("bhqf,bhfd->bhqd", phi_q, kv)
    den = jnp.einsum("bhqf,bhf->bhq", phi_q, z)[..., None] + 1e-6
    o = num / den
    return (lambda x, *d: x.transpose(*d))(o, 0, 2, 1, 3).reshape(B, S, D) @ wo
```

```python
import jax
import jax.numpy as jnp
import jax.experimental.pallas as pl
import jax.experimental.pallas.tpu as pltpu

_H = 32
_DH = 32
_TS = 512
_NT = (((1,), (1,)), ((), ()))


def _dual_softmax_t(pT, ts):
    p3 = pT.reshape(_H, _DH, ts)
    mx = jnp.max(p3, axis=1, keepdims=True)
    mn = jnp.min(p3, axis=1, keepdims=True)
    ep = jnp.exp(p3 - mx)
    en = jnp.exp(mn - p3)
    php = ep * (1.0 / jnp.sum(ep, axis=1, keepdims=True))
    phn = en * (1.0 / jnp.sum(en, axis=1, keepdims=True))
    return php.reshape(_H * _DH, ts), phn.reshape(_H * _DH, ts)


def _kernel(x_ref, wqkv_ref, wphi_ref, wo_ref, o_ref,
            wkT_ref, wqT_ref, kvp_ref, kvn_ref, zp_ref, zn_ref, lhs_ref):
    ph = pl.program_id(0)
    i = pl.program_id(1)
    ns = pl.num_programs(1)
    D = _H * _DH
    ts = x_ref.shape[0]
    f32 = jnp.float32
    bf16 = jnp.bfloat16
    row = jax.lax.broadcasted_iota(jnp.int32, (128, 128), 0)
    col = jax.lax.broadcasted_iota(jnp.int32, (128, 128), 1)
    bd_mask = (row // _DH) == (col // _DH)

    @pl.when((ph == 0) & (i == 0))
    def _fold():
        for g in range(8):
            w = wphi_ref[128 * g:128 * (g + 1), :].astype(f32)
            wt = jnp.concatenate([w, w, w, w], axis=1)
            bdT = jnp.where(bd_mask, wt, 0.0).T.astype(bf16)
            wq_g = wqkv_ref[:, 128 * g:128 * (g + 1)]
            wk_g = wqkv_ref[:, D + 128 * g:D + 128 * (g + 1)]
            wqT_ref[128 * g:128 * (g + 1), :] = jax.lax.dot_general(
                bdT, wq_g, _NT, preferred_element_type=f32).astype(bf16)
            wkT_ref[128 * g:128 * (g + 1), :] = jax.lax.dot_general(
                bdT, wk_g, _NT, preferred_element_type=f32).astype(bf16)
        kvp_ref[...] = jnp.zeros_like(kvp_ref)
        kvn_ref[...] = jnp.zeros_like(kvn_ref)
        zp_ref[...] = jnp.zeros_like(zp_ref)
        zn_ref[...] = jnp.zeros_like(zn_ref)

    @pl.when(ph == 0)
    def _phase_k():
        x = x_ref[...]
        pT = jax.lax.dot_general(wkT_ref[...], x, _NT, preferred_element_type=f32)
        v = jnp.dot(x, wqkv_ref[:, 2 * D:3 * D], preferred_element_type=f32).astype(bf16)
        php, phn = _dual_softmax_t(pT, ts)
        zp = php[:, 0:128]
        zn = phn[:, 0:128]
        for j in range(1, ts // 128):
            zp = zp + php[:, 128 * j:128 * (j + 1)]
            zn = zn + phn[:, 128 * j:128 * (j + 1)]
        zp_ref[...] += zp
        zn_ref[...] += zn
        php = php.astype(bf16)
        phn = phn.astype(bf16)
        for g in range(8):
            sl = slice(128 * g, 128 * (g + 1))
            kvp_ref[sl, :] += jnp.dot(php[sl, :], v[:, sl], preferred_element_type=f32)
            kvn_ref[sl, :] += jnp.dot(phn[sl, :], v[:, sl], preferred_element_type=f32)

    @pl.when((ph == 1) & (i == 0))
    def _build_lhs():
        zsel = col == (row // _DH)
        for g in range(8):
            sl = slice(128 * g, 128 * (g + 1))
            for half, (kv_ref, z_ref) in enumerate(((kvp_ref, zp_ref), (kvn_ref, zn_ref))):
                kvT = jnp.where(bd_mask, kv_ref[sl, :], 0.0).T
                z = jnp.sum(z_ref[sl, :], axis=1, keepdims=True)
                zT = jnp.where(zsel, z, 0.0).T
                lhs_ref[g, 0:128, 128 * half:128 * (half + 1)] = kvT.astype(bf16)
                lhs_ref[g, 128:144, 128 * half:128 * (half + 1)] = zT[0:16, :].astype(bf16)

    @pl.when(ph == 1)
    def _phase_q():
        x = x_ref[...]
        pT = jax.lax.dot_general(wqT_ref[...], x, _NT, preferred_element_type=f32)
        php, phn = _dual_softmax_t(pT, ts)
        php = php.astype(bf16)
        phn = phn.astype(bf16)
        outs = []
        for g in range(8):
            sl = slice(128 * g, 128 * (g + 1))
            phi = jnp.concatenate([php[sl, :], phn[sl, :]], axis=0)
            res = jnp.dot(lhs_ref[g], phi, preferred_element_type=f32)
            for j in range(4):
                den = res[128 + j:129 + j, :] + 1e-6
                outs.append(res[_DH * j:_DH * (j + 1), :] * (1.0 / den))
        oT = jnp.concatenate(outs, axis=0)
        o = oT.T.astype(bf16)
        o_ref[...] = jnp.dot(o, wo_ref[...], preferred_element_type=f32).astype(o_ref.dtype)


@jax.jit
def pallas_standalone__linear_kernel_hedgehog__prompt_kernel(x, wqkv, w_phi, wo):
    B, S, D = x.shape
    ts = _TS
    ns = S // ts
    x2 = x.reshape(S, D)
    wphi2 = w_phi.reshape(_H * _DH, _DH)
    out = pl.pallas_call(
        _kernel,
        grid=(2, ns),
        in_specs=[
            pl.BlockSpec((ts, D), lambda p, i: (i, 0)),
            pl.BlockSpec((D, 3 * D), lambda p, i: (0, 0)),
            pl.BlockSpec((_H * _DH, _DH), lambda p, i: (0, 0)),
            pl.BlockSpec((D, D), lambda p, i: (0, 0)),
        ],
        out_specs=pl.BlockSpec((ts, D), lambda p, i: (p * i, 0)),
        out_shape=jax.ShapeDtypeStruct((S, D), x.dtype),
        scratch_shapes=[
            pltpu.VMEM((D, D), jnp.bfloat16),
            pltpu.VMEM((D, D), jnp.bfloat16),
            pltpu.VMEM((D, 128), jnp.float32),
            pltpu.VMEM((D, 128), jnp.float32),
            pltpu.VMEM((D, 128), jnp.float32),
            pltpu.VMEM((D, 128), jnp.float32),
            pltpu.VMEM((8, 144, 256), jnp.bfloat16),
        ],
        compiler_params=pltpu.CompilerParams(
            dimension_semantics=("arbitrary", "arbitrary"),
            vmem_limit_bytes=100 * 1024 * 1024,
        ),
    )(x2, wqkv, wphi2, wo)
    return out.reshape(B, S, D)
```

```python
import jax
import jax.numpy as jnp
import jax.experimental.pallas as pl
import jax.experimental.pallas.tpu as pltpu

_H = 32
_DH = 32
_TS = 512
_NT = (((1,), (1,)), ((), ()))
_NCH = 4
_NOC = 4


def _dual_softmax_t(pT, ts):
    p3 = pT.reshape(_H, _DH, ts)
    mx = jnp.max(p3, axis=1, keepdims=True)
    mn = jnp.min(p3, axis=1, keepdims=True)
    ep = jnp.exp(p3 - mx)
    en = jnp.exp(mn - p3)
    php = ep * (1.0 / jnp.sum(ep, axis=1, keepdims=True))
    phn = en * (1.0 / jnp.sum(en, axis=1, keepdims=True))
    return php.reshape(_H * _DH, ts), phn.reshape(_H * _DH, ts)


def _kernel(x_hbm, wqkv_hbm, wphi_hbm, wo_hbm, o_hbm,
            wphi_ref, obuf_ref, osem, x_ref, w_ref, wo_ref, wkT_ref, wqT_ref, kvp_ref, kvn_ref, zp_ref, zn_ref, lhs_ref, sems):
    ph = pl.program_id(0)
    i = pl.program_id(1)
    D = _H * _DH
    S = x_ref.shape[0]
    ts = _TS
    ns = S // ts
    f32 = jnp.float32
    bf16 = jnp.bfloat16
    cw = D // _NCH
    row = jax.lax.broadcasted_iota(jnp.int32, (128, 128), 0)
    col = jax.lax.broadcasted_iota(jnp.int32, (128, 128), 1)
    bd_mask = (row // _DH) == (col // _DH)

    def wk_copy(c):
        lo = D + c * cw
        return pltpu.make_async_copy(wqkv_hbm.at[:, lo:lo + cw], w_ref.at[:, lo:lo + cw], sems.at[c])

    def wv_copy():
        return pltpu.make_async_copy(wqkv_hbm.at[:, 2 * D:3 * D], w_ref.at[:, 2 * D:3 * D], sems.at[_NCH])

    def wq_copy():
        return pltpu.make_async_copy(wqkv_hbm.at[:, 0:D], w_ref.at[:, 0:D], sems.at[_NCH + 1])

    def wo_copy():
        return pltpu.make_async_copy(wo_hbm, wo_ref, sems.at[_NCH + 2])

    def wphi_copy():
        return pltpu.make_async_copy(wphi_hbm, wphi_ref, sems.at[_NCH + 3 + ns])

    def x_copy(j):
        r = pl.ds(pl.multiple_of(j * ts, ts), ts)
        return pltpu.make_async_copy(x_hbm.at[r, :], x_ref.at[r, :], sems.at[_NCH + 3 + j])

    def fold_group(g, m, dst_ref):
        w = wphi_ref[128 * g:128 * (g + 1), :].astype(f32)
        wt = jnp.concatenate([w, w, w, w], axis=1)
        bdT = jnp.where(bd_mask, wt, 0.0).T.astype(bf16)
        w_g = w_ref[:, m * D + 128 * g:m * D + 128 * (g + 1)]
        dst_ref[128 * g:128 * (g + 1), :] = jax.lax.dot_general(
            bdT, w_g, _NT, preferred_element_type=f32).astype(bf16)

    def k_step(first):
        x = x_ref[pl.ds(pl.multiple_of(i * ts, ts), ts), :]
        pT = jax.lax.dot_general(wkT_ref[...], x, _NT, preferred_element_type=f32)
        php, phn = _dual_softmax_t(pT, ts)
        zp = php[:, 0:128]
        zn = phn[:, 0:128]
        for j in range(1, ts // 128):
            zp = zp + php[:, 128 * j:128 * (j + 1)]
            zn = zn + phn[:, 128 * j:128 * (j + 1)]
        if first:
            zp_ref[...] = zp
            zn_ref[...] = zn
        else:
            zp_ref[...] += zp
            zn_ref[...] += zn
        php = php.astype(bf16)
        phn = phn.astype(bf16)
        if first:
            wv_copy().wait()
        v = jnp.dot(x, w_ref[:, 2 * D:3 * D], preferred_element_type=f32).astype(bf16)
        for g in range(8):
            sl = slice(128 * g, 128 * (g + 1))
            kvp = jnp.dot(php[sl, :], v[:, sl], preferred_element_type=f32)
            kvn = jnp.dot(phn[sl, :], v[:, sl], preferred_element_type=f32)
            if first:
                kvp_ref[sl, :] = kvp
                kvn_ref[sl, :] = kvn
            else:
                kvp_ref[sl, :] += kvp
                kvn_ref[sl, :] += kvn
        if first:
            wq_copy().wait()
            for g in range(8):
                fold_group(g, 0, wqT_ref)

    @pl.when((ph == 0) & (i == 0))
    def _first():
        wphi_copy().start()
        for c in range(_NCH):
            wk_copy(c).start()
        x_copy(0).start()
        wv_copy().start()
        wq_copy().start()
        for j in range(1, ns):
            x_copy(j).start()
        wo_copy().start()
        wphi_copy().wait()
        for c in range(_NCH):
            wk_copy(c).wait()
            for g in range(c * cw // 128, (c + 1) * cw // 128):
                fold_group(g, 1, wkT_ref)
        x_copy(0).wait()
        k_step(True)

    @pl.when((ph == 0) & (i > 0))
    def _phase_k():
        x_copy(i).wait()
        k_step(False)

    @pl.when((ph == 1) & (i == 0))
    def _build_lhs():
        wo_copy().wait()
        eye = (row == col).astype(bf16)
        ones = jnp.ones((16, 128), bf16)
        zmask = (jax.lax.broadcasted_iota(jnp.int32, (16, 128), 1) // _DH) == \
            jax.lax.broadcasted_iota(jnp.int32, (16, 128), 0)
        for g in range(8):
            sl = slice(128 * g, 128 * (g + 1))
            for half, (kv_ref, z_ref) in enumerate(((kvp_ref, zp_ref), (kvn_ref, zn_ref))):
                kv = jnp.where(bd_mask, kv_ref[sl, :], 0.0).astype(bf16)
                kvT = jax.lax.dot_general(eye, kv, _NT, preferred_element_type=f32)
                zT = jax.lax.dot_general(ones, z_ref[sl, :].astype(bf16), _NT,
                                         preferred_element_type=f32)
                lhs_ref[g, 0:128, 128 * half:128 * (half + 1)] = kvT.astype(bf16)
                lhs_ref[g, 128:144, 128 * half:128 * (half + 1)] = jnp.where(zmask, zT, 0.0).astype(bf16)

    @pl.when(ph == 1)
    def _phase_q():
        x = x_ref[pl.ds(pl.multiple_of(i * ts, ts), ts), :]
        pT = jax.lax.dot_general(wqT_ref[...], x, _NT, preferred_element_type=f32)
        php, phn = _dual_softmax_t(pT, ts)
        php = php.astype(bf16)
        phn = phn.astype(bf16)
        outs = []
        for g in range(8):
            sl = slice(128 * g, 128 * (g + 1))
            phi = jnp.concatenate([php[sl, :], phn[sl, :]], axis=0)
            res = jnp.dot(lhs_ref[g], phi, preferred_element_type=f32)
            for j in range(4):
                den = res[128 + j:129 + j, :] + 1e-6
                outs.append(res[_DH * j:_DH * (j + 1), :] * (1.0 / den))
        oT = jnp.concatenate(outs, axis=0)
        o = oT.T.astype(bf16)
        rows = pl.ds(pl.multiple_of(i * ts, ts), ts)
        for c in range(_NOC):
            cs = slice(c * (D // _NOC), (c + 1) * (D // _NOC))
            obuf_ref[rows, cs] = jnp.dot(o, wo_ref[:, cs], preferred_element_type=f32).astype(bf16)
            pltpu.make_async_copy(obuf_ref.at[rows, cs], o_hbm.at[rows, cs], osem).start()

    @pl.when((ph == 1) & (i == ns - 1))
    def _drain():
        pltpu.make_async_copy(obuf_ref, o_hbm, osem).wait()


@jax.jit
def pallas_standalone__linear_kernel_hedgehog__prompt_kernel(x, wqkv, w_phi, wo):
    B, S, D = x.shape
    ts = _TS
    ns = S // ts
    x2 = x.reshape(S, D)
    wphi2 = w_phi.reshape(_H * _DH, _DH)
    out = pl.pallas_call(
        _kernel,
        grid=(2, ns),
        in_specs=[
            pl.BlockSpec(memory_space=pl.ANY),
            pl.BlockSpec(memory_space=pl.ANY),
            pl.BlockSpec(memory_space=pl.ANY),
            pl.BlockSpec(memory_space=pl.ANY),
        ],
        out_specs=pl.BlockSpec(memory_space=pl.ANY),
        out_shape=jax.ShapeDtypeStruct((S, D), x.dtype),
        scratch_shapes=[
            pltpu.VMEM((_H * _DH, _DH), jnp.bfloat16),
            pltpu.VMEM((S, D), jnp.bfloat16),
            pltpu.SemaphoreType.DMA(()),
            pltpu.VMEM((S, D), jnp.bfloat16),
            pltpu.VMEM((D, 3 * D), jnp.bfloat16),
            pltpu.VMEM((D, D), jnp.bfloat16),
            pltpu.VMEM((D, D), jnp.bfloat16),
            pltpu.VMEM((D, D), jnp.bfloat16),
            pltpu.VMEM((D, 128), jnp.float32),
            pltpu.VMEM((D, 128), jnp.float32),
            pltpu.VMEM((D, 128), jnp.float32),
            pltpu.VMEM((D, 128), jnp.float32),
            pltpu.VMEM((8, 144, 256), jnp.bfloat16),
            pltpu.SemaphoreType.DMA((_NCH + 4 + ns,)),
        ],
        compiler_params=pltpu.CompilerParams(
            dimension_semantics=("arbitrary", "arbitrary"),
            vmem_limit_bytes=100 * 1024 * 1024,
        ),
    )(x2, wqkv, wphi2, wo)
    return out.reshape(B, S, D)
```

```python
import jax
import jax.numpy as jnp
import jax.experimental.pallas as pl
import jax.experimental.pallas.tpu as pltpu

_H = 32
_DH = 32
_TS = 512
_NCH = 2
_NOC = 8
_NT = (((1,), (1,)), ((), ()))


def _dual_softmax_t(pT):
    r, ts = pT.shape
    p3 = pT.reshape(r // _DH, _DH, ts)
    mx = jnp.max(p3, axis=1, keepdims=True)
    mn = jnp.min(p3, axis=1, keepdims=True)
    ep = jnp.exp(p3 - mx)
    en = jnp.exp(mn - p3)
    php = ep * (1.0 / jnp.sum(ep, axis=1, keepdims=True))
    phn = en * (1.0 / jnp.sum(en, axis=1, keepdims=True))
    return php.reshape(r, ts), phn.reshape(r, ts)


def _lane_fold(a):
    acc = a[:, 0:128]
    for j in range(1, a.shape[1] // 128):
        acc = acc + a[:, 128 * j:128 * (j + 1)]
    return acc


def _kernel(x_hbm, wqkv_hbm, wphi_hbm, wo_hbm, o_hbm,
            wphi_ref, bdT_ref, obuf_ref, osem, x_ref, w_ref, wo_ref, wkT_ref, wqT_ref,
            kvp_ref, kvn_ref, zp_ref, zn_ref, lhs_ref, sems):
    ph = pl.program_id(0)
    i = pl.program_id(1)
    D = _H * _DH
    S = x_ref.shape[0]
    ts = _TS
    ns = S // ts
    f32 = jnp.float32
    bf16 = jnp.bfloat16
    cw = D // _NCH
    ng = D // 128
    row = jax.lax.broadcasted_iota(jnp.int32, (128, 128), 0)
    col = jax.lax.broadcasted_iota(jnp.int32, (128, 128), 1)
    bd_mask = (row // _DH) == (col // _DH)

    def wk_copy(c):
        lo = D + c * cw
        return pltpu.make_async_copy(wqkv_hbm.at[:, lo:lo + cw], w_ref.at[:, lo:lo + cw], sems.at[c])

    def wv_copy():
        return pltpu.make_async_copy(wqkv_hbm.at[:, 2 * D:3 * D], w_ref.at[:, 2 * D:3 * D], sems.at[_NCH])

    def wq_copy():
        return pltpu.make_async_copy(wqkv_hbm.at[:, 0:D], w_ref.at[:, 0:D], sems.at[_NCH + 1])

    def wo_copy():
        return pltpu.make_async_copy(wo_hbm, wo_ref, sems.at[_NCH + 2])

    def wphi_copy():
        return pltpu.make_async_copy(wphi_hbm, wphi_ref, sems.at[_NCH + 3])

    def x0_copy(h):
        r = slice(h * (ts // 2), (h + 1) * (ts // 2))
        return pltpu.make_async_copy(x_hbm.at[r, :], x_ref.at[r, :], sems.at[_NCH + 4 + h])

    def x_copy(j):
        r = pl.ds(pl.multiple_of(j * ts, ts), ts)
        return pltpu.make_async_copy(x_hbm.at[r, :], x_ref.at[r, :], sems.at[_NCH + 5 + j])

    def fold_group(g, m, dst_ref):
        w_g = w_ref[:, m * D + 128 * g:m * D + 128 * (g + 1)]
        dst_ref[128 * g:128 * (g + 1), :] = jax.lax.dot_general(
            bdT_ref[g], w_g, _NT, preferred_element_type=f32).astype(bf16)

    @pl.when((ph == 0) & (i == 0))
    def _first():
        wphi_copy().start()
        wk_copy(0).start()
        x0_copy(0).start()
        x0_copy(1).start()
        for c in range(1, _NCH):
            wk_copy(c).start()
        wphi_copy().wait()
        for g in range(ng):
            w = wphi_ref[128 * g:128 * (g + 1), :].astype(f32)
            wt = jnp.concatenate([w, w, w, w], axis=1)
            bdT_ref[g] = jnp.where(bd_mask, wt, 0.0).T.astype(bf16)

        def fold_chunk(c):
            for g in range(c * cw // 128, (c + 1) * cw // 128):
                fold_group(g, 1, wkT_ref)

        def softmax_chunk(c, pT):
            php, phn = _dual_softmax_t(pT)
            zp_ref[c * cw:(c + 1) * cw, :] = _lane_fold(php)
            zn_ref[c * cw:(c + 1) * cw, :] = _lane_fold(phn)
            return php.astype(bf16), phn.astype(bf16)

        wk_copy(0).wait()
        fold_chunk(0)
        x0_copy(0).wait()
        pa = jax.lax.dot_general(wkT_ref[0:cw, :], x_ref[0:ts // 2, :], _NT, preferred_element_type=f32)
        x0_copy(1).wait()
        wk_copy(1).wait()
        wv_copy().start()
        pb = jax.lax.dot_general(wkT_ref[0:cw, :], x_ref[ts // 2:ts, :], _NT, preferred_element_type=f32)
        phis = [softmax_chunk(0, jnp.concatenate([pa, pb], axis=1))]
        fold_chunk(1)
        phis.append(softmax_chunk(1, jax.lax.dot_general(
            wkT_ref[cw:2 * cw, :], x_ref[0:ts, :], _NT, preferred_element_type=f32)))
        wq_copy().start()
        for j in range(1, ns):
            x_copy(j).start()
        wo_copy().start()
        wv_copy().wait()
        v = jnp.dot(x_ref[0:ts, :], w_ref[:, 2 * D:3 * D], preferred_element_type=f32).astype(bf16)
        gpc = cw // 128
        for g in range(ng):
            sl = slice(128 * g, 128 * (g + 1))
            php, phn = phis[g // gpc]
            lsl = slice(128 * (g % gpc), 128 * (g % gpc + 1))
            kvp_ref[sl, :] = jnp.dot(php[lsl, :], v[:, sl], preferred_element_type=f32)
            kvn_ref[sl, :] = jnp.dot(phn[lsl, :], v[:, sl], preferred_element_type=f32)
        wq_copy().wait()
        for g in range(ng):
            fold_group(g, 0, wqT_ref)

    @pl.when((ph == 0) & (i > 0))
    def _phase_k():
        x_copy(i).wait()
        x = x_ref[pl.ds(pl.multiple_of(i * ts, ts), ts), :]
        pT = jax.lax.dot_general(wkT_ref[...], x, _NT, preferred_element_type=f32)
        php, phn = _dual_softmax_t(pT)
        zp_ref[...] += _lane_fold(php)
        zn_ref[...] += _lane_fold(phn)
        php = php.astype(bf16)
        phn = phn.astype(bf16)
        v = jnp.dot(x, w_ref[:, 2 * D:3 * D], preferred_element_type=f32).astype(bf16)
        for g in range(ng):
            sl = slice(128 * g, 128 * (g + 1))
            kvp_ref[sl, :] += jnp.dot(php[sl, :], v[:, sl], preferred_element_type=f32)
            kvn_ref[sl, :] += jnp.dot(phn[sl, :], v[:, sl], preferred_element_type=f32)

    @pl.when((ph == 1) & (i == 0))
    def _build_lhs():
        wo_copy().wait()
        eye = (row == col).astype(bf16)
        ones = jnp.ones((16, 128), bf16)
        zmask = (jax.lax.broadcasted_iota(jnp.int32, (16, 128), 1) // _DH) == \
            jax.lax.broadcasted_iota(jnp.int32, (16, 128), 0)
        for g in range(ng):
            sl = slice(128 * g, 128 * (g + 1))
            for half, (kv_ref, z_ref) in enumerate(((kvp_ref, zp_ref), (kvn_ref, zn_ref))):
                kv = jnp.where(bd_mask, kv_ref[sl, :], 0.0).astype(bf16)
                kvT = jax.lax.dot_general(eye, kv, _NT, preferred_element_type=f32)
                zT = jax.lax.dot_general(ones, z_ref[sl, :].astype(bf16), _NT,
                                         preferred_element_type=f32)
                lhs_ref[g, 0:128, 128 * half:128 * (half + 1)] = kvT.astype(bf16)
                lhs_ref[g, 128:144, 128 * half:128 * (half + 1)] = jnp.where(zmask, zT, 0.0).astype(bf16)

    @pl.when(ph == 1)
    def _phase_q():
        rows = pl.ds(pl.multiple_of(i * ts, ts), ts)
        x = x_ref[rows, :]
        pT = jax.lax.dot_general(wqT_ref[...], x, _NT, preferred_element_type=f32)
        php, phn = _dual_softmax_t(pT)
        php = php.astype(bf16)
        phn = phn.astype(bf16)
        outs = []
        for g in range(ng):
            sl = slice(128 * g, 128 * (g + 1))
            phi = jnp.concatenate([php[sl, :], phn[sl, :]], axis=0)
            res = jnp.dot(lhs_ref[g], phi, preferred_element_type=f32)
            for j in range(4):
                den = res[128 + j:129 + j, :] + 1e-6
                outs.append(res[_DH * j:_DH * (j + 1), :] * (1.0 / den))
        o = jnp.concatenate(outs, axis=0).T.astype(bf16)
        for c in range(_NOC):
            cs = slice(c * (D // _NOC), (c + 1) * (D // _NOC))
            obuf_ref[rows, cs] = jnp.dot(o, wo_ref[:, cs], preferred_element_type=f32).astype(bf16)
            pltpu.make_async_copy(obuf_ref.at[rows, cs], o_hbm.at[rows, cs], osem).start()

    @pl.when((ph == 1) & (i == ns - 1))
    def _drain():
        pltpu.make_async_copy(obuf_ref, o_hbm, osem).wait()


@jax.jit
def pallas_standalone__linear_kernel_hedgehog__prompt_kernel(x, wqkv, w_phi, wo):
    B, S, D = x.shape
    assert B == 1 and D == _H * _DH and S % _TS == 0
    ns = S // _TS
    bf16 = jnp.bfloat16
    out = pl.pallas_call(
        _kernel,
        grid=(2, ns),
        in_specs=[pl.BlockSpec(memory_space=pl.ANY)] * 4,
        out_specs=pl.BlockSpec(memory_space=pl.ANY),
        out_shape=jax.ShapeDtypeStruct((S, D), bf16),
        scratch_shapes=[
            pltpu.VMEM((_H * _DH, _DH), bf16),
            pltpu.VMEM((D // 128, 128, 128), bf16),
            pltpu.VMEM((S, D), bf16),
            pltpu.SemaphoreType.DMA(()),
            pltpu.VMEM((S, D), bf16),
            pltpu.VMEM((D, 3 * D), bf16),
            pltpu.VMEM((D, D), bf16),
            pltpu.VMEM((D, D), bf16),
            pltpu.VMEM((D, D), bf16),
            pltpu.VMEM((D, 128), jnp.float32),
            pltpu.VMEM((D, 128), jnp.float32),
            pltpu.VMEM((D, 128), jnp.float32),
            pltpu.VMEM((D, 128), jnp.float32),
            pltpu.VMEM((D // 128, 144, 256), bf16),
            pltpu.SemaphoreType.DMA((_NCH + 5 + ns,)),
        ],
        compiler_params=pltpu.CompilerParams(
            dimension_semantics=("arbitrary", "arbitrary"),
            vmem_limit_bytes=100 * 1024 * 1024,
        ),
    )(x.reshape(S, D).astype(bf16), wqkv.astype(bf16),
      w_phi.reshape(_H * _DH, _DH).astype(bf16), wo.astype(bf16))
    return out.reshape(B, S, D).astype(x.dtype)
```
